```python
import os as _os
_os.environ.setdefault("JAX_PLATFORMS", "cpu")
import jax
import jax.numpy as jnp

def _softmax(x, axis=-1):
    return jax.nn.softmax(x, axis=axis)
def _gelu(x):
    return jax.nn.gelu(x, approximate=True)
def _silu(x):
    return jax.nn.silu(x)
def _sigmoid(x):
    return jax.nn.sigmoid(x)
def _layernorm(x, axis=-1, eps=1e-5):
    m = jnp.mean(x, axis=axis, keepdims=True)
    v = jnp.var(x, axis=axis, keepdims=True)
    return (x - m) / jnp.sqrt(v + eps)
def _scatter_add(tgt, idx, src, axis=0):
    return tgt.at[idx].add(src)
def _segment_sum(src, seg, n):
    return jax.ops.segment_sum(src, seg, n)
class _Rng:
    def __init__(self, key):
        self._k = key
    def _next(self):
        self._k, sub = jax.random.split(self._k)
        return sub
    def normal(self, shape):
        return jax.random.normal(self._next(), shape, dtype=jnp.bfloat16)
    def randint(self, lo, hi, shape):
        return jax.random.randint(self._next(), shape, lo, hi, dtype=jnp.int32)
    def uniform(self, shape, lo=0.0, hi=1.0):
        return jax.random.uniform(self._next(), shape, jnp.bfloat16, lo, hi)
    def permutation(self, n):
        return jax.random.permutation(self._next(), n)


kernel_name = 'concat_heads__sliding_block_cached__compressed_kv_cla__decode'

def setup_inputs():
    _rng = _Rng(jax.random.key(int.from_bytes(__import__("os").urandom(4), "little")))
    _w = (lambda a: (lambda t: t.astype(jnp.bfloat16) if jnp.issubdtype(t.dtype, jnp.floating) else t)(jnp.asarray(a)))
    def _A_setup():
        B, Sq, D = 1, 1, 512
        Hq, Hkv, Sk, Dh = 32, 32, 4096, 128
        assert Hq % Hkv == 0, (Hq, Hkv)
        return {
            "x": _w((lambda *s: _rng.normal(s) * 0.8)(B, Sq, D)),
            "k_cache": _w((lambda *s: _rng.normal(s) * 0.8)(B, Hkv, Sk, Dh)),
            "v_cache": _w((lambda *s: _rng.normal(s) * 0.05)(B, Hkv, Sk, Dh)),
            "wq": _w((lambda *s: _rng.normal(s) * 0.8)(D, Hq * Dh) * (D ** -0.5)),
            "wo": _w((lambda *s: _rng.normal(s) * 0.05)(Hq * Dh, D) * ((Hq * Dh) ** -0.5)),
        }
    _A_in = _A_setup()

    def _B_setup():
        B, H, Sq, Sk, D, M = 1, 32, 1, 4096, 128, 512
        Dc = 4 * D
        return {
            "x": _w((lambda *s: _rng.normal(s) * 1.6)(B, Sq, M)),
            "c_kv": _w((lambda *s: _rng.normal(s) * 0.1)(B, Sk, Dc)),
            "w_q": _w((lambda *s: _rng.normal(s) * 1.6)(M, H, D) * (M ** -0.5)),
            "w_uk": _w((lambda *s: _rng.normal(s) * 1.6)(Dc, H, D) * (Dc ** -0.5)),
            "w_uv": _w((lambda *s: _rng.normal(s) * 0.1)(Dc, H, D) * (Dc ** -0.5)),
            "w_o": _w((lambda *s: _rng.normal(s) * 0.1)(H, D, M) * ((H * D) ** -0.5)),
        }
    _B_in = _B_setup()

    return {
        "A_x": _A_in["x"],
        "A_k_cache": _A_in["k_cache"],
        "A_v_cache": _A_in["v_cache"],
        "A_wq": _A_in["wq"],
        "A_wo": _A_in["wo"],
        "B_x": _B_in["x"],
        "B_c_kv": _B_in["c_kv"],
        "B_w_q": _B_in["w_q"],
        "B_w_uk": _B_in["w_uk"],
        "B_w_uv": _B_in["w_uv"],
        "B_w_o": _B_in["w_o"],
    }

def reference(A_x, A_k_cache, A_v_cache, A_wq, A_wo, B_x, B_c_kv, B_w_q, B_w_uk, B_w_uv, B_w_o):
    def _A_ref(x, k_cache, v_cache, wq, wo):
        B, Sq, D = x.shape
        Hq, Dh = 32, 128
        Hkv, Sk = k_cache.shape[1], k_cache.shape[2]
        W = min(4096, max(256, Sk // 4))
        rep = Hq // Hkv
        q = (lambda x, *d: x.transpose(*d))((x @ wq).reshape(B, Sq, Hq, Dh), 0, 2, 1, 3)
        k = jnp.repeat(k_cache[:, :, Sk - W:, :], rep, axis=1)
        v = jnp.repeat(v_cache[:, :, Sk - W:, :], rep, axis=1)
        scores = jnp.einsum("bhqd,bhkd->bhqk", q, k) * (Dh ** -0.5)
        p = _softmax(scores, axis=-1)
        o = jnp.einsum("bhqk,bhkd->bhqd", p, v)
        return (lambda x, *d: x.transpose(*d))(o, 0, 2, 1, 3).reshape(B, Sq, Hq * Dh) @ wo

    def _B_ref(x, c_kv, w_q, w_uk, w_uv, w_o):
        B, Sq, M = x.shape[0], x.shape[1], x.shape[2]
        Sk = c_kv.shape[1]
        H, D = w_q.shape[1], w_q.shape[2]
        q = jnp.einsum("bqm,mhd->bhqd", x, w_q)
        k = jnp.einsum("bkc,chd->bhkd", c_kv, w_uk)
        v = jnp.einsum("bkc,chd->bhkd", c_kv, w_uv)
        scores = jnp.einsum("bhqd,bhkd->bhqk", q, k) * (D ** -0.5)
        off = Sk - Sq
        qi = jnp.arange(Sq)[:, None]
        kj = jnp.arange(Sk)[None, :]
        cmask = kj <= (qi + off)
        scores = jnp.where(cmask[None, None], scores, -1e9)
        p = _softmax(scores, axis=-1)
        ctx = jnp.einsum("bhqk,bhkd->bhqd", p, v)
        return jnp.einsum("bhqd,hdm->bqm", ctx, w_o)

    a = _A_ref(A_x, A_k_cache, A_v_cache, A_wq, A_wo)
    b = _B_ref(B_x, B_c_kv, B_w_q, B_w_uk, B_w_uv, B_w_o)
    return jnp.concatenate([a, b], axis=-1)
```

```python
import functools
import jax
import jax.numpy as jnp
from jax import lax
import jax.experimental.pallas as pl
import jax.experimental.pallas.tpu as pltpu

BF = jnp.bfloat16
F32 = jnp.float32
H, DH, DM, SK, WIN, DC = 32, 128, 512, 4096, 1024, 512
NT = (((1,), (1,)), ((), ()))


def _dot(a, b):
    return jnp.dot(a, b, preferred_element_type=F32)


def _dot_nt(a, b):
    return lax.dot_general(a, b, NT, preferred_element_type=F32)


def _kernel(xa_h, k_h, v_h, wq_h, wo_h, xb_h, c_h, bq_h, uk_h, uv_h, bo_h,
            out_ref,
            xa, xb, kb, vb, wqb, wob, cb, bqb, ukb, uvb, bob,
            xr_s, qabs_s, sb_s, z_s, ctx_s, qa_s, sa_s, oa_s, sems, *, tail, nsem, compute):
    groups = [
        [(bq_h, bqb), (xb_h, xb), (xa_h, xa)],
        [(uk_h, ukb)],
        [(wq_h, wqb)],
        [(c_h.at[0], cb)],
        [(k_h.at[0, pl.ds(0, 16), pl.ds(SK - WIN, WIN)], kb.at[pl.ds(0, 16)])],
        [(k_h.at[0, pl.ds(16, 16), pl.ds(SK - WIN, WIN)], kb.at[pl.ds(16, 16)])],
        [(v_h.at[0, pl.ds(0, 16), pl.ds(SK - WIN, WIN)], vb.at[pl.ds(0, 16)])],
        [(v_h.at[0, pl.ds(16, 16), pl.ds(SK - WIN, WIN)], vb.at[pl.ds(16, 16)])],
        [(uv_h, uvb)],
        [(bo_h, bob)],
    ]
    r0 = 0
    for n in tail:
        groups.append([(wo_h.at[pl.ds(r0, n)], wob.at[pl.ds(r0, n)])])
        r0 += n
    assert r0 == H * DH
    cps = [[pltpu.make_async_copy(s, d, sems.at[i % nsem]) for (s, d) in g] for i, g in enumerate(groups)]
    state = {"next": 0}

    def start_next():
        i = state["next"]
        if i < len(cps):
            for c in cps[i]:
                c.start()
            state["next"] = i + 1

    def arrive(i):
        for c in cps[i]:
            c.wait()
        start_next()

    for _ in range(nsem):
        start_next()

    row = lax.broadcasted_iota(jnp.int32, (16, 128), 0)
    lane = lax.broadcasted_iota(jnp.int32, (16, 128), 1)
    diag = (lane & 15) == row
    scale = DH ** -0.5

    arrive(0)
    if compute:
        x4 = xb[0].astype(F32)
        d = jnp.concatenate(
            [jnp.where((lane >> 3) == row, jnp.broadcast_to(x4[:, 128 * b:128 * (b + 1)], (16, 128)), 0.0)
             for b in range(4)], axis=0).astype(BF)
        rr = lax.broadcasted_iota(jnp.int32, (128, 128), 0)
        rc = lax.broadcasted_iota(jnp.int32, (128, 128), 1)
        rep = jnp.where((rr & 7) == (rc >> 4), 1.0, 0.0).astype(BF)
        xr_s[...] = _dot(d, rep)

        def bq_body(i, carry):
            lhs = jnp.concatenate(
                [jnp.where(diag, jnp.broadcast_to(xr_s[pl.ds(8 * i + u, 1), :], (16, 128)), 0.0).astype(BF)
                 for u in range(8)], axis=1)
            m0 = pl.multiple_of(64 * i, 64)
            return tuple(
                carry[g] + _dot(lhs, bqb[pl.ds(m0, 64), 16 * g:16 * (g + 1), :].reshape(1024, 128))
                for g in range(2))

        qb = lax.fori_loop(0, 8, bq_body, (jnp.zeros((16, 128), F32),) * 2)
        qb = [q.astype(BF) for q in qb]

    arrive(1)
    if compute:
        def qabs_body(b, _):
            for g in range(2):
                acc = jnp.zeros((16, 128), F32)
                for t in range(16):
                    w = ukb[b, :, t, 16 * g:16 * (g + 1), :].reshape(128, 128)
                    o = jnp.where(diag, _dot_nt(qb[g], w), 0.0)
                    acc = acc + (pltpu.roll(o, t, 1) if t else o)
                for bit in (1, 2, 4, 8):
                    acc = jnp.where((row & bit) != 0, pltpu.roll(acc, 128 - bit, 1), acc)
                qabs_s[b, 16 * g:16 * (g + 1), :] = acc.astype(BF)
            return 0

        lax.fori_loop(0, 4, qabs_body, 0)

    arrive(2)
    if compute:
        xa16 = jnp.broadcast_to(xa[0].astype(F32), (16, DM)).astype(BF)

        def qa_body(j, _):
            c0 = pl.multiple_of(512 * j, 512)
            q = _dot(xa16, wqb[:, pl.ds(c0, 512)])
            for u in range(4):
                qa_s[4 * j + u] = q[:, 128 * u:128 * (u + 1)].astype(BF)
            return 0

        lax.fori_loop(0, 8, qa_body, 0)

    arrive(3)
    if compute:
        qabs = jnp.concatenate([qabs_s[b] for b in range(4)], axis=1)

        def sb_body(i, m):
            k0 = pl.multiple_of(512 * i, 512)
            s = _dot_nt(qabs, cb[pl.ds(k0, 512), :]) * scale
            sb_s[i] = s
            for u in range(4):
                m = jnp.maximum(m, s[:, 128 * u:128 * (u + 1)])
            return m

        m = lax.fori_loop(0, 8, sb_body, jnp.full((32, 128), -jnp.inf, F32))
        m = jnp.max(m, axis=1, keepdims=True)

        def pb_body(i, carry):
            l, acc = carry
            k0 = pl.multiple_of(512 * i, 512)
            p = jnp.exp(sb_s[i] - m)
            for u in range(4):
                l = l + p[:, 128 * u:128 * (u + 1)]
            return l, acc + _dot(p.astype(BF), cb[pl.ds(k0, 512), :])

        l, acc = lax.fori_loop(0, 8, pb_body, (jnp.zeros((32, 128), F32), jnp.zeros((32, DC), F32)))
        cc = acc / jnp.sum(l, axis=1, keepdims=True)
        for b in range(4):
            for g in range(2):
                z_s[b, 16 * g:16 * (g + 1), :] = pltpu.roll(
                    cc[16 * g:16 * (g + 1), 128 * b:128 * (b + 1)], 0, 1, stride=1, stride_axis=0)

    for g in range(2):
        arrive(4 + g)
        if compute:
            def sa_body(i, _):
                for u in range(2):
                    h = 16 * g + 2 * i + u
                    s = _dot_nt(qa_s[h], kb[h])
                    sa_s[pl.ds(h, 1), :] = s[0:1, :]
                return 0

            lax.fori_loop(0, 8, sa_body, 0)
            s = sa_s[16 * g:16 * (g + 1), :] * scale
            p = jnp.exp(s - jnp.max(s, axis=1, keepdims=True))
            sa_s[16 * g:16 * (g + 1), :] = p / jnp.sum(p, axis=1, keepdims=True)

    for g in range(2):
        arrive(6 + g)
        if compute:
            pg = sa_s[16 * g:16 * (g + 1), :].astype(BF)

            def pa_body(i, o):
                for u in range(2):
                    hl = 2 * i + u
                    o = jnp.where(row == hl, _dot(pg, vb[16 * g + hl]), o)
                return o

            oa_s[16 * g:16 * (g + 1), :] = lax.fori_loop(0, 8, pa_body, jnp.zeros((16, 128), F32))

    arrive(8)
    if compute:
        def ctx_body(b, carry):
            res = []
            for g in range(2):
                z = z_s[b, 16 * g:16 * (g + 1), :]
                acc = carry[g]
                for t in range(16):
                    zt = pltpu.roll(z, 128 - t, 1) if t else z
                    lhs = jnp.where(diag, zt, 0.0).astype(BF)
                    acc = acc + _dot(lhs, uvb[b, :, t, 16 * g:16 * (g + 1), :].reshape(128, 128))
                res.append(acc)
            return tuple(res)

        ctx = lax.fori_loop(0, 4, ctx_body, (jnp.zeros((16, 128), F32),) * 2)
        for g in range(2):
            ctx_s[16 * g:16 * (g + 1), :] = ctx[g]

    def head_lhs(src, h):
        return jnp.broadcast_to(src[pl.ds(h, 1), :], (16, 128)).astype(BF)

    def proj(src, wbuf, h0, nh, acc):
        nloop, rem = divmod(nh, 4)
        if nloop > 1:
            def body(i, acc):
                lhs = jnp.concatenate([head_lhs(src, h0 + 4 * i + u) for u in range(4)], axis=1)
                r = pl.multiple_of(128 * h0 + 512 * i, 128)
                return acc + _dot(lhs, wbuf[pl.ds(r, 512), :])
            acc = lax.fori_loop(0, nloop, body, acc)
            h0 += 4 * nloop
        else:
            rem = nh
        if rem:
            lhs = jnp.concatenate([head_lhs(src, h0 + u) for u in range(rem)], axis=1)
            acc = acc + _dot(lhs, wbuf[pl.ds(128 * h0, 128 * rem), :])
        return acc

    arrive(9)
    if compute:
        acc = proj(ctx_s, bob, 0, H, jnp.zeros((16, DM), F32))
        out_ref[0, :, DM:2 * DM] = acc[0:1, :].astype(BF)

    acc = jnp.zeros((16, DM), F32)
    r0 = 0
    for i, n in enumerate(tail):
        arrive(10 + i)
        if compute:
            if n % 128 == 0 and r0 % 128 == 0:
                acc = proj(oa_s, wob, r0 // 128, n // 128, acc)
            else:
                h, off = divmod(r0, 128)
                assert off + n <= 128
                acc = acc + _dot(head_lhs(oa_s, h)[:, off:off + n], wob[pl.ds(r0, n), :])
        r0 += n
    if compute:
        out_ref[0, :, 0:DM] = acc[0:1, :].astype(BF)
    else:
        out_ref[...] = jnp.zeros(out_ref.shape, BF)


def make(tail=(2048, 1280, 512, 128, 128), nsem=3, compute=True, **cp):
    def fn(A_x, A_k_cache, A_v_cache, A_wq, A_wo, B_x, B_c_kv, B_w_q, B_w_uk, B_w_uv, B_w_o):
        return pl.pallas_call(
            functools.partial(_kernel, tail=tail, nsem=nsem, compute=compute),
            out_shape=jax.ShapeDtypeStruct((1, 1, 2 * DM), BF),
            in_specs=[pl.BlockSpec(memory_space=pl.ANY)] * 11,
            scratch_shapes=[
                pltpu.VMEM((1, 1, DM), BF), pltpu.VMEM((1, 1, DM), BF),
                pltpu.VMEM((H, WIN, DH), BF), pltpu.VMEM((H, WIN, DH), BF),
                pltpu.VMEM((DM, H * DH), BF), pltpu.VMEM((H * DH, DM), BF), pltpu.VMEM((SK, DC), BF),
                pltpu.VMEM((DM, H, DH), BF), pltpu.VMEM((4, 8, 16, H, DH), BF), pltpu.VMEM((4, 8, 16, H, DH), BF),
                pltpu.VMEM((H * DH, DM), BF),
                pltpu.VMEM((64, 128), F32), pltpu.VMEM((4, 32, 128), BF), pltpu.VMEM((8, 32, 512), F32),
                pltpu.VMEM((4, 32, 128), F32), pltpu.VMEM((H, DH), F32),
                pltpu.VMEM((H, 16, 128), BF), pltpu.VMEM((H, WIN), F32), pltpu.VMEM((H, DH), F32),
                pltpu.SemaphoreType.DMA((nsem,)),
            ],
            compiler_params=pltpu.CompilerParams(vmem_limit_bytes=100 * 1024 * 1024, **cp),
        )(A_x, A_k_cache, A_v_cache, A_wq, A_wo, B_x, B_c_kv, B_w_q,
          B_w_uk.reshape(4, 8, 16, H, DH), B_w_uv.reshape(4, 8, 16, H, DH), B_w_o.reshape(H * DH, DM))
    return fn

@jax.jit
def pallas_concat_heads__sliding_block_cached__compressed_kv_cla__decode_kernel(
    A_x, A_k_cache, A_v_cache, A_wq, A_wo, B_x, B_c_kv, B_w_q, B_w_uk, B_w_uv, B_w_o,
):
    return make()(A_x, A_k_cache, A_v_cache, A_wq, A_wo, B_x, B_c_kv, B_w_q, B_w_uk, B_w_uv, B_w_o)
```

```python
import jax
import jax.numpy as jnp
from jax import lax
import jax.experimental.pallas as pl
import jax.experimental.pallas.tpu as pltpu

BF16 = jnp.bfloat16
F32 = jnp.float32

H = 32
DH = 128
DM = 512
SK = 4096
WIN = min(4096, max(256, SK // 4))
DC = 512
G = 16
KC = 512

WO_MXU_ROWS = (2048, 1152, 512, 256)
WO_VPU_ROWS = (64, 48, 16)
NUM_INPUT_DMAS = 12 + len(WO_MXU_ROWS) + len(WO_VPU_ROWS)


def _dot(a, b):
    return jnp.dot(a, b, preferred_element_type=F32)


def _dot_nt(a, b):
    return lax.dot_general(a, b, (((1,), (1,)), ((), ())), preferred_element_type=F32)


def _project(src, w, h0, nh, acc):
    def lhs(first, count):
        return jnp.concatenate(
            [jnp.broadcast_to(src[pl.ds(first + u, 1), :], (G, DH)).astype(BF16)
             for u in range(count)], axis=1)

    steps = nh // 4 if nh >= 8 else 0
    if steps:
        def body(i, acc):
            r0 = pl.multiple_of(DH * (h0 + 4 * i), DH)
            return acc + _dot(lhs(h0 + 4 * i, 4), w[pl.ds(r0, 4 * DH), :])

        acc = lax.fori_loop(0, steps, body, acc)
    h1, rest = h0 + 4 * steps, nh - 4 * steps
    if rest:
        acc = acc + _dot(lhs(h1, rest), w[pl.ds(DH * h1, DH * rest), :])
    return acc


def _stream_and_compute(
        xa_hbm, k_hbm, v_hbm, wq_hbm, wo_hbm, xb_hbm, c_hbm, bq_hbm, uk_hbm, uv_hbm, bo_hbm,
        xa, k, v, wq, wo, xb, c, bq, uk, uv, bo,
        xrep_s, qabs_s, sb_s, lat_s, ctx_s, qa_s, pa_s, oa_s, ocol_s, out_s,
        sems):
    window = pl.ds(SK - WIN, WIN)
    pairs = [(bq_hbm, bq), (xb_hbm, xb), (xa_hbm, xa), (uk_hbm, uk), (wq_hbm, wq), (c_hbm.at[0], c)]
    for src, dst in ((k_hbm, k), (v_hbm, v)):
        pairs += [(src.at[0, pl.ds(G * g, G), window], dst.at[pl.ds(G * g, G)]) for g in range(2)]
    pairs += [(uv_hbm, uv), (bo_hbm, bo)]
    r0 = 0
    for n in WO_MXU_ROWS + WO_VPU_ROWS:
        pairs.append((wo_hbm.at[pl.ds(r0, n)], wo.at[pl.ds(r0, n)]))
        r0 += n
    assert r0 == H * DH and sum(WO_VPU_ROWS) == DH and len(pairs) == NUM_INPUT_DMAS
    copies = [pltpu.make_async_copy(src, dst, sems.at[i]) for i, (src, dst) in enumerate(pairs)]
    for copy in copies:
        copy.start()
    bq_dma, xb_dma, xa_dma, uk_dma, wq_dma, c_dma = copies[:6]
    k_dma, v_dma, (uv_dma, bo_dma), wo_dma = copies[6:8], copies[8:10], copies[10:12], copies[12:]

    row = lax.broadcasted_iota(jnp.int32, (G, 128), 0)
    lane = lax.broadcasted_iota(jnp.int32, (G, 128), 1)
    diag = (lane & (G - 1)) == row
    scale = DH ** -0.5

    bq_dma.wait()
    xb_dma.wait()
    x = xb[0].astype(F32)
    picked = jnp.concatenate(
        [jnp.where((lane >> 3) == row, jnp.broadcast_to(x[:, 128 * b:128 * (b + 1)], (G, 128)), 0.0)
         for b in range(DM // 128)], axis=0).astype(BF16)
    src_lane = lax.broadcasted_iota(jnp.int32, (128, 128), 0)
    dst_lane = lax.broadcasted_iota(jnp.int32, (128, 128), 1)
    spread = jnp.where((src_lane & 7) == (dst_lane >> 4), 1.0, 0.0).astype(BF16)
    xrep_s[...] = _dot(picked, spread)

    def bq_body(i, acc):
        lhs = jnp.concatenate(
            [jnp.where(diag, jnp.broadcast_to(xrep_s[pl.ds(8 * i + u, 1), :], (G, 128)), 0.0).astype(BF16)
             for u in range(8)], axis=1)
        m0 = pl.multiple_of(64 * i, 64)
        return tuple(
            acc[g] + _dot(lhs, bq[pl.ds(m0, 64), G * g:G * (g + 1), :].reshape(64 * G, DH))
            for g in range(2))

    qb = lax.fori_loop(0, DM // 64, bq_body, (jnp.zeros((G, DH), F32),) * 2)
    qb = [q.astype(BF16) for q in qb]

    uk_dma.wait()

    def qabs_body(b, carry):
        for g in range(2):
            acc = jnp.zeros((G, 128), F32)
            for t in range(16):
                tile = uk[b, :, t, G * g:G * (g + 1), :].reshape(128, DH)
                part = jnp.where(diag, _dot_nt(qb[g], tile), 0.0)
                acc = acc + (pltpu.roll(part, t, 1) if t else part)
            for bit in (1, 2, 4, 8):
                acc = jnp.where((row & bit) != 0, pltpu.roll(acc, 128 - bit, 1), acc)
            qabs_s[b, G * g:G * (g + 1), :] = acc.astype(BF16)
        return carry

    lax.fori_loop(0, DC // 128, qabs_body, 0)

    wq_dma.wait()
    xa_dma.wait()
    xa_rows = jnp.broadcast_to(xa[0].astype(F32), (G, DM)).astype(BF16)

    def qa_body(i, carry):
        q = _dot(xa_rows, wq[:, pl.ds(pl.multiple_of(4 * DH * i, 4 * DH), 4 * DH)])
        for u in range(4):
            qa_s[4 * i + u] = q[:, DH * u:DH * (u + 1)].astype(BF16)
        return carry

    lax.fori_loop(0, H // 4, qa_body, 0)

    c_dma.wait()
    qabs = jnp.concatenate([qabs_s[b] for b in range(DC // 128)], axis=1)

    def scores_body(i, m):
        s = _dot_nt(qabs, c[pl.ds(pl.multiple_of(KC * i, KC), KC), :]) * scale
        sb_s[i] = s
        for u in range(KC // 128):
            m = jnp.maximum(m, s[:, 128 * u:128 * (u + 1)])
        return m

    m = lax.fori_loop(0, SK // KC, scores_body, jnp.full((H, 128), -jnp.inf, F32))
    m = jnp.max(m, axis=1, keepdims=True)

    def latent_body(i, carry):
        denom, acc = carry
        p = jnp.exp(sb_s[i] - m)
        for u in range(KC // 128):
            denom = denom + p[:, 128 * u:128 * (u + 1)]
        return denom, acc + _dot(p.astype(BF16), c[pl.ds(pl.multiple_of(KC * i, KC), KC), :])

    denom, acc = lax.fori_loop(
        0, SK // KC, latent_body, (jnp.zeros((H, 128), F32), jnp.zeros((H, DC), F32)))
    lat = acc / jnp.sum(denom, axis=1, keepdims=True)
    for b in range(DC // 128):
        for g in range(2):
            lat_s[b, G * g:G * (g + 1), :] = pltpu.roll(
                lat[G * g:G * (g + 1), 128 * b:128 * (b + 1)], 0, 1, stride=1, stride_axis=0)

    for g in range(2):
        k_dma[g].wait()

        def sa_body(i, carry, g=g):
            for u in range(2):
                h = G * g + 2 * i + u
                pa_s[pl.ds(h, 1), :] = _dot_nt(qa_s[h], k[h])[0:1, :]
            return carry

        lax.fori_loop(0, G // 2, sa_body, 0)
        s = pa_s[G * g:G * (g + 1), :] * scale
        p = jnp.exp(s - jnp.max(s, axis=1, keepdims=True))
        pa_s[G * g:G * (g + 1), :] = p / jnp.sum(p, axis=1, keepdims=True)

    for g in range(2):
        v_dma[g].wait()
        p = pa_s[G * g:G * (g + 1), :].astype(BF16)

        def oa_body(i, o, g=g, p=p):
            for u in range(2):
                j = 2 * i + u
                o = jnp.where(row == j, _dot(p, v[G * g + j]), o)
            return o

        oa_s[G * g:G * (g + 1), :] = lax.fori_loop(0, G // 2, oa_body, jnp.zeros((G, DH), F32))

    uv_dma.wait()

    def ctx_body(b, carry):
        out = []
        for g in range(2):
            skewed = lat_s[b, G * g:G * (g + 1), :]
            acc = carry[g]
            for t in range(16):
                shifted = pltpu.roll(skewed, 128 - t, 1) if t else skewed
                tile = uv[b, :, t, G * g:G * (g + 1), :].reshape(128, DH)
                acc = acc + _dot(jnp.where(diag, shifted, 0.0).astype(BF16), tile)
            out.append(acc)
        return tuple(out)

    ctx = lax.fori_loop(0, DC // 128, ctx_body, (jnp.zeros((G, DH), F32),) * 2)
    for g in range(2):
        ctx_s[G * g:G * (g + 1), :] = ctx[g]

    bo_dma.wait()
    acc = _project(ctx_s, bo, 0, H, jnp.zeros((G, DM), F32))
    out_s[0, :, DM:2 * DM] = acc[0:1, :].astype(BF16)

    o_last = oa_s[H - 1:H, :].astype(BF16).astype(F32)
    ocol_s[...] = jnp.broadcast_to(o_last, (DH, DH)).T

    acc = jnp.zeros((G, DM), F32)
    r0 = 0
    for dma, n in zip(wo_dma, WO_MXU_ROWS):
        dma.wait()
        acc = _project(oa_s, wo, r0 // DH, n // DH, acc)
        r0 += n
    partial = []
    for i, (dma, n) in enumerate(zip(wo_dma[len(WO_MXU_ROWS):], WO_VPU_ROWS)):
        if i == len(WO_VPU_ROWS) - 1:
            first_row = lax.broadcasted_iota(jnp.int32, (8, DM), 0) == 0
            partial = [partial[0] + jnp.where(first_row, acc[0:8, :], 0.0)]
        dma.wait()
        ocol = ocol_s[pl.ds(r0 - (H - 1) * DH, n), :]
        prod = wo[pl.ds(r0, n), :].astype(F32) * jnp.concatenate([ocol] * (DM // 128), axis=1)
        partial = [prod[8 * u:8 * (u + 1), :] for u in range(n // 8)] + partial
        while len(partial) > 1:
            partial = [partial[u] + partial[u + 1] if u + 1 < len(partial) else partial[u]
                       for u in range(0, len(partial), 2)]
        r0 += n
    out_s[0, :, 0:DM] = jnp.sum(partial[0], axis=0, keepdims=True).astype(BF16)


def _kernel(*refs):
    inputs, out_hbm, scratch, out_sem = refs[:11], refs[11], refs[12:-1], refs[-1]
    out_dma = pltpu.make_async_copy(scratch[-1], out_hbm, out_sem)

    def scoped(sems):
        _stream_and_compute(*inputs, *scratch, sems)
        out_dma.start()

    pl.run_scoped(scoped, pltpu.SemaphoreType.DMA((NUM_INPUT_DMAS,)))
    out_dma.wait()


@jax.jit
def pallas_concat_heads__sliding_block_cached__compressed_kv_cla__decode_kernel(
    A_x: jax.Array,
    A_k_cache: jax.Array,
    A_v_cache: jax.Array,
    A_wq: jax.Array,
    A_wo: jax.Array,
    B_x: jax.Array,
    B_c_kv: jax.Array,
    B_w_q: jax.Array,
    B_w_uk: jax.Array,
    B_w_uv: jax.Array,
    B_w_o: jax.Array,
):
    assert A_x.shape == B_x.shape == (1, 1, DM)
    assert A_k_cache.shape == A_v_cache.shape == (1, H, SK, DH)
    assert B_c_kv.shape == (1, SK, DC)
    up_shape = (DC // 128, 8, 16, H, DH)
    hbm = pl.BlockSpec(memory_space=pltpu.HBM)

    return pl.pallas_call(
        _kernel,
        out_shape=jax.ShapeDtypeStruct((1, 1, 2 * DM), BF16),
        in_specs=[hbm] * 11,
        out_specs=hbm,
        scratch_shapes=[
            pltpu.VMEM((1, 1, DM), BF16),
            pltpu.VMEM((H, WIN, DH), BF16),
            pltpu.VMEM((H, WIN, DH), BF16),
            pltpu.VMEM((DM, H * DH), BF16),
            pltpu.VMEM((H * DH, DM), BF16),
            pltpu.VMEM((1, 1, DM), BF16),
            pltpu.VMEM((SK, DC), BF16),
            pltpu.VMEM((DM, H, DH), BF16),
            pltpu.VMEM(up_shape, BF16),
            pltpu.VMEM(up_shape, BF16),
            pltpu.VMEM((H * DH, DM), BF16),
            pltpu.VMEM((DM // 8, 128), F32),
            pltpu.VMEM((DC // 128, H, 128), BF16),
            pltpu.VMEM((SK // KC, H, KC), F32),
            pltpu.VMEM((DC // 128, H, 128), F32),
            pltpu.VMEM((H, DH), F32),
            pltpu.VMEM((H, G, DH), BF16),
            pltpu.VMEM((H, WIN), F32),
            pltpu.VMEM((H, DH), F32),
            pltpu.VMEM((DH, DH), F32),
            pltpu.VMEM((1, 1, 2 * DM), BF16),
            pltpu.SemaphoreType.DMA(()),
        ],
        compiler_params=pltpu.CompilerParams(vmem_limit_bytes=64 * 1024 * 1024),
    )(
        A_x, A_k_cache, A_v_cache, A_wq, A_wo, B_x, B_c_kv, B_w_q,
        B_w_uk.reshape(up_shape), B_w_uv.reshape(up_shape), B_w_o.reshape(H * DH, DM),
    )
```

```python
import functools

import jax
import jax.numpy as jnp
from jax import lax
import jax.experimental.pallas as pl
import jax.experimental.pallas.tpu as pltpu

BF16 = jnp.bfloat16
F32 = jnp.float32

H, DH, DM, SK, DC, G, KC = 32, 128, 512, 4096, 512, 16, 512
WIN = min(4096, max(256, SK // 4))
NS, NT = 8, 16
S_BQ, S_X, S_UK, S_WQ, S_C, S_K, S_V, S_UV, S_BO, S_WO = 0, 1, 2, 3, 4, 5, 7, 9, 10, 11


def _dot(a, b):
    return jnp.dot(a, b, preferred_element_type=F32)


def _dot_nt(a, b):
    return lax.dot_general(a, b, (((1,), (1,)), ((), ())), preferred_element_type=F32)


def _mult(x, n):
    return x if isinstance(x, int) else pl.multiple_of(x, n)


def _stream_and_compute(
        xa_hbm, k_hbm, v_hbm, wq_hbm, wo_hbm, xb_hbm, c_hbm, bq_hbm, uk_hbm, uv_hbm, bo_hbm,
        xa, k, v, wq, wo, xb, c, bq, uk, uv, bo,
        xrep_s, qb_s, qabs_s, sb_s, lat_s, ctx_s, qa_s, pa_s, oa_s, operm_s, ocol_s, out_s,
        sems, *, tail_steps, vpu_groups, skip, feed_first, sorder):

    def start(src, dst, sem, j):
        pltpu.make_async_copy(src, dst, sems.at[sem]).start(priority=j % 2)

    def wait(buf, sem):
        pltpu.make_async_copy(buf, buf, sems.at[sem]).wait()

    def feed_rows(src, dst, n, sem, t):
        for j, s in enumerate(sorder):
            r = pl.ds(_mult((s * NT + t) * n, n), n)
            start(src.at[r], dst.at[r], sem, j)

    def feed_up(src, dst, sem, t):
        for j, s in enumerate(sorder):
            idx = (s // 2, 4 * (s % 2) + (t >> 2), pl.ds(4 * (t & 3), 4))
            start(src.at[idx], dst.at[idx], sem, j)

    def feed_wq(i):
        for half in range(2):
            for j, s in enumerate(sorder):
                idx = (pl.ds(_mult(64 * s + 8 * i, 8), 8), pl.ds(2048 * half, 2048))
                start(wq_hbm.at[idx], wq.at[idx], S_WQ, j)

    def feed_window(src, dst, sem, t, h0, n):
        r = _mult(t * 128, 128)
        for j in range(n):
            start(src.at[0, h0 + j, pl.ds(SK - WIN + r, 128)], dst.at[h0 + j, pl.ds(r, 128)], sem, j)

    def feed_wo(sem, t, j0=0, n=NS):
        for j in range(j0, j0 + n):
            start(wo_hbm.at[pl.ds(_mult((sorder[j] * NT + t) * 32, 32), 32)], wo.at[t, j], sem, j)

    def loop(n, name, feed, body, init):
        def step(i, carry):
            if feed_first:
                feed(i)
            if name not in skip:
                carry = body(i, carry)
            if not feed_first:
                feed(i)
            return carry
        return lax.fori_loop(0, n, step, init)

    xb_dma = pltpu.make_async_copy(xb_hbm, xb, sems.at[S_X])
    xa_dma = pltpu.make_async_copy(xa_hbm, xa, sems.at[S_X])
    loop(NT, "", lambda t: feed_rows(bq_hbm, bq, 4, S_BQ, t), lambda i, cy: cy, 0)
    xb_dma.start()
    xa_dma.start()
    loop(NT, "", lambda t: feed_up(uk_hbm, uk, S_UK, t), lambda i, cy: cy, 0)

    row = lax.broadcasted_iota(jnp.int32, (G, 128), 0)
    lane = lax.broadcasted_iota(jnp.int32, (G, 128), 1)
    diag = (lane & (G - 1)) == row
    scale = DH ** -0.5

    wait(bq, S_BQ)
    xb_dma.wait()
    xa_dma.wait()
    x = xb[0].astype(F32)
    picked = jnp.concatenate(
        [jnp.where((lane >> 3) == row, jnp.broadcast_to(x[:, 128 * b:128 * (b + 1)], (G, 128)), 0.0)
         for b in range(DM // 128)], axis=0).astype(BF16)
    src_lane = lax.broadcasted_iota(jnp.int32, (128, 128), 0)
    dst_lane = lax.broadcasted_iota(jnp.int32, (128, 128), 1)
    spread = jnp.where((src_lane & 7) == (dst_lane >> 4), 1.0, 0.0).astype(BF16)
    xrep_s[...] = _dot(picked, spread)

    def bq_body(i, acc):
        lhs = jnp.concatenate(
            [jnp.where(diag, jnp.broadcast_to(xrep_s[pl.ds(8 * i + u, 1), :], (G, 128)), 0.0).astype(BF16)
             for u in range(8)], axis=1)
        m0 = pl.multiple_of(64 * i, 64)
        return tuple(
            acc[g] + _dot(lhs, bq[pl.ds(m0, 64), G * g:G * (g + 1), :].reshape(64 * G, DH))
            for g in range(2))

    qb = loop(8, "bq", feed_wq, bq_body, (jnp.zeros((G, DH), F32),) * 2)
    for g in range(2):
        qb_s[g] = qb[g].astype(BF16)

    wait(uk, S_UK)

    def qabs_body(i, carry):
        b, g = i >> 1, i & 1
        heads = pl.ds(pl.multiple_of(G * g, G), G)
        q = qb_s[g]
        acc = jnp.zeros((G, 128), F32)
        for t in range(16):
            tile = uk[b, :, t, heads, :].reshape(128, DH)
            part = jnp.where(diag, _dot_nt(q, tile), 0.0)
            acc = acc + (pltpu.roll(part, t, 1) if t else part)
        for bit in (1, 2, 4, 8):
            acc = jnp.where((row & bit) != 0, pltpu.roll(acc, 128 - bit, 1), acc)
        qabs_s[b, heads, :] = acc.astype(BF16)
        return carry

    loop(8, "qabs", lambda i: [feed_rows(c_hbm.at[0], c, 32, S_C, 2 * i + u) for u in range(2)], qabs_body, 0)

    wait(wq, S_WQ)
    xa_rows = jnp.broadcast_to(xa[0].astype(F32), (G, DM)).astype(BF16)

    def qa_body(i, carry):
        q = _dot(xa_rows, wq[:, pl.ds(pl.multiple_of(4 * DH * i, 4 * DH), 4 * DH)])
        for u in range(4):
            qa_s[4 * i + u] = q[:, DH * u:DH * (u + 1)].astype(BF16)
        return carry

    loop(8, "qa", lambda i: feed_window(k_hbm, k, S_K, i, 0, G), qa_body, 0)

    wait(c, S_C)
    qabs = jnp.concatenate([qabs_s[b] for b in range(DC // 128)], axis=1)

    def scores_body(i, m):
        s = _dot_nt(qabs, c[pl.ds(pl.multiple_of(KC * i, KC), KC), :]) * scale
        sb_s[i] = s
        for u in range(KC // 128):
            m = jnp.maximum(m, s[:, 128 * u:128 * (u + 1)])
        return m

    m = loop(8, "sb", lambda i: feed_window(k_hbm, k, S_K + 1, i >> 1, G + 8 * (i & 1), 8),
             scores_body, jnp.full((H, 128), -jnp.inf, F32))
    m = jnp.max(m, axis=1, keepdims=True)

    def latent_body(i, carry):
        denom, acc = carry
        p = jnp.exp(sb_s[i] - m)
        for u in range(KC // 128):
            denom = denom + p[:, 128 * u:128 * (u + 1)]
        return denom, acc + _dot(p.astype(BF16), c[pl.ds(pl.multiple_of(KC * i, KC), KC), :])

    denom, acc = loop(8, "lat", lambda i: feed_window(k_hbm, k, S_K + 1, 4 + (i >> 1), G + 8 * (i & 1), 8),
                      latent_body, (jnp.zeros((H, 128), F32), jnp.zeros((H, DC), F32)))
    lat = acc / jnp.sum(denom, axis=1, keepdims=True)
    for b in range(DC // 128):
        for g in range(2):
            lat_s[b, G * g:G * (g + 1), :] = pltpu.roll(
                lat[G * g:G * (g + 1), 128 * b:128 * (b + 1)], 0, 1, stride=1, stride_axis=0)

    for g in range(2):
        wait(k.at[pl.ds(G * g, G)], S_K + g)

        def sa_body(i, carry, g=g):
            for u in range(2):
                h = G * g + 2 * i + u
                pa_s[pl.ds(h, 1), :] = _dot_nt(qa_s[h], k[h])[0:1, :]
            return carry

        loop(8, "sa", lambda i, g=g: feed_window(v_hbm, v, S_V + g, i, G * g, G), sa_body, 0)
        s = pa_s[G * g:G * (g + 1), :] * scale
        p = jnp.exp(s - jnp.max(s, axis=1, keepdims=True))
        pa_s[G * g:G * (g + 1), :] = p / jnp.sum(p, axis=1, keepdims=True)

    for g in range(2):
        wait(v.at[pl.ds(G * g, G)], S_V + g)
        p = pa_s[G * g:G * (g + 1), :].astype(BF16)

        def oa_body(i, o, g=g, p=p):
            for u in range(2):
                j = 2 * i + u
                o = jnp.where(row == j, _dot(p, v[G * g + j]), o)
            return o

        feed = ((lambda i: [feed_up(uv_hbm, uv, S_UV, 2 * i + u) for u in range(2)]) if g == 0 else
                (lambda i: [feed_rows(bo_hbm, bo, 32, S_BO, 2 * i + u) for u in range(2)]))
        oa_s[G * g:G * (g + 1), :] = loop(8, "oa", feed, oa_body, jnp.zeros((G, DH), F32))

    def operm_body(u, carry):
        for sb in range(2):
            src = [jnp.broadcast_to(oa_s[pl.ds(4 * sorder[4 * sb + i] + u, 1), :], (G, DH)) for i in range(4)]
            for q in range(4):
                blk = None
                for i in range(4):
                    shift = (32 * (i - q)) % 128
                    piece = pltpu.roll(src[i], shift, 1) if shift else src[i]
                    blk = piece if blk is None else jnp.where((lane >> 5) == i, piece, blk)
                operm_s[4 * u + q, :, 128 * sb:128 * (sb + 1)] = blk.astype(BF16)
        return carry

    lax.fori_loop(0, 4, operm_body, 0)
    last = operm_s[NT - 1].astype(F32)[0:1, :]
    for sb in range(2):
        ocol_s[128 * sb:128 * (sb + 1), :] = jnp.broadcast_to(last[:, 128 * sb:128 * (sb + 1)], (DH, DH)).T

    wait(uv, S_UV)
    ctx_s[...] = jnp.zeros((H, DH), F32)

    def ctx_body(i, carry):
        b, g = i >> 1, i & 1
        heads = pl.ds(pl.multiple_of(G * g, G), G)
        skewed = lat_s[b, heads, :]
        acc = ctx_s[heads, :]
        for t in range(16):
            shifted = pltpu.roll(skewed, 128 - t, 1) if t else skewed
            tile = uv[b, :, t, heads, :].reshape(128, DH)
            acc = acc + _dot(jnp.where(diag, shifted, 0.0).astype(BF16), tile)
        ctx_s[heads, :] = acc
        return carry

    loop(8, "ctx", lambda i: feed_wo(S_WO + (i >> 2), i), ctx_body, 0)

    wait(bo, S_BO)

    def bo_body(i, acc):
        lhs = jnp.concatenate(
            [jnp.broadcast_to(ctx_s[pl.ds(4 * i + u, 1), :], (G, DH)).astype(BF16) for u in range(4)], axis=1)
        return acc + _dot(lhs, bo[pl.ds(pl.multiple_of(4 * DH * i, 4 * DH), 4 * DH), :])

    def feed_bo(i):
        for jj in range(4):
            j = 4 * (i & 1) + jj
            s = sorder[jj] + (sorder[4 + jj] - sorder[jj]) * (i & 1)
            t = 8 + (i >> 1)
            start(wo_hbm.at[pl.ds(pl.multiple_of((s * NT + t) * 32, 32), 32)], wo.at[t, j], S_WO + 2, jj)

    acc = loop(8, "bo", feed_bo, bo_body, jnp.zeros((G, DM), F32))
    t0 = 12
    for i, n in enumerate(tail_steps):
        for t in range(t0, t0 + n):
            feed_wo(S_WO + 3 + i, t)
        t0 += n
    assert t0 == NT - 1
    j0 = 0
    for i, n in enumerate(vpu_groups):
        feed_wo(S_WO + 3 + len(tail_steps) + i, t0, j0, n)
        j0 += n
    assert j0 == NS
    out_s[0, :, DM:2 * DM] = acc[0:1, :].astype(BF16)

    acc = jnp.zeros((G, DM), F32)
    t0 = 0
    for i, n in enumerate((4, 4, 4) + tail_steps):
        wait(wo.at[pl.ds(t0, n)], S_WO + i)
        if "wo" not in skip:
            lhs = jnp.concatenate([operm_s[t] for t in range(t0, t0 + n)], axis=1)
            acc = acc + _dot(lhs, wo[t0:t0 + n].reshape(n * NS * 32, DM))
        t0 += n
    partial = []
    j0 = 0
    for i, n in enumerate(vpu_groups):
        if i == len(vpu_groups) - 1:
            first_row = lax.broadcasted_iota(jnp.int32, (8, DM), 0) == 0
            seed = jnp.where(first_row, acc[0:8, :], 0.0)
            partial = [partial[0] + seed] if partial else [seed]
        wait(wo.at[t0, pl.ds(j0, n)], S_WO + 3 + len(tail_steps) + i)
        ocol = ocol_s[32 * j0:32 * (j0 + n), :]
        prod = wo[t0, j0:j0 + n].reshape(32 * n, DM).astype(F32) * jnp.concatenate([ocol] * (DM // 128), axis=1)
        partial = [prod[8 * u:8 * (u + 1), :] for u in range(4 * n)] + partial
        while len(partial) > 1:
            partial = [partial[u] + partial[u + 1] if u + 1 < len(partial) else partial[u]
                       for u in range(0, len(partial), 2)]
        j0 += n
    out_s[0, :, 0:DM] = jnp.sum(partial[0], axis=0, keepdims=True).astype(BF16)


def _kernel(*refs, nsem, **kw):
    inputs, out_hbm, scratch, out_sem = refs[:11], refs[11], refs[12:-1], refs[-1]
    out_dma = pltpu.make_async_copy(scratch[-1], out_hbm, out_sem)

    def scoped(sems):
        _stream_and_compute(*inputs, *scratch, sems, **kw)
        out_dma.start()

    pl.run_scoped(scoped, pltpu.SemaphoreType.DMA((nsem,)))
    out_dma.wait()


def run(A_x, A_k_cache, A_v_cache, A_wq, A_wo, B_x, B_c_kv, B_w_q, B_w_uk, B_w_uv, B_w_o, *,
        tail_steps=(2, 1), vpu_groups=(2, 2, 2, 2), skip=(), feed_first=True, sorder=tuple(range(8)), **cp):
    up_shape = (DC // 128, 8, 16, H, DH)
    hbm = pl.BlockSpec(memory_space=pltpu.HBM)
    return pl.pallas_call(
        functools.partial(_kernel, nsem=S_WO + 3 + len(tail_steps) + len(vpu_groups), tail_steps=tail_steps,
                          vpu_groups=vpu_groups, skip=skip, feed_first=feed_first, sorder=sorder),
        out_shape=jax.ShapeDtypeStruct((1, 1, 2 * DM), BF16),
        in_specs=[hbm] * 11,
        out_specs=hbm,
        scratch_shapes=[
            pltpu.VMEM((1, 1, DM), BF16), pltpu.VMEM((H, WIN, DH), BF16), pltpu.VMEM((H, WIN, DH), BF16),
            pltpu.VMEM((DM, H * DH), BF16), pltpu.VMEM((NT, NS, 32, DM), BF16), pltpu.VMEM((1, 1, DM), BF16),
            pltpu.VMEM((SK, DC), BF16), pltpu.VMEM((DM, H, DH), BF16), pltpu.VMEM(up_shape, BF16),
            pltpu.VMEM(up_shape, BF16), pltpu.VMEM((H * DH, DM), BF16),
            pltpu.VMEM((DM // 8, 128), F32), pltpu.VMEM((2, G, DH), BF16), pltpu.VMEM((DC // 128, H, 128), BF16),
            pltpu.VMEM((SK // KC, H, KC), F32), pltpu.VMEM((DC // 128, H, 128), F32), pltpu.VMEM((H, DH), F32),
            pltpu.VMEM((H, G, DH), BF16), pltpu.VMEM((H, WIN), F32), pltpu.VMEM((H, DH), F32),
            pltpu.VMEM((NT, G, 256), BF16), pltpu.VMEM((256, DH), F32), pltpu.VMEM((1, 1, 2 * DM), BF16),
            pltpu.SemaphoreType.DMA(()),
        ],
        compiler_params=pltpu.CompilerParams(vmem_limit_bytes=64 * 1024 * 1024, **cp),
    )(A_x, A_k_cache, A_v_cache, A_wq, A_wo, B_x, B_c_kv, B_w_q,
      B_w_uk.reshape(up_shape), B_w_uv.reshape(up_shape), B_w_o.reshape(H * DH, DM))


@jax.jit
def pallas_concat_heads__sliding_block_cached__compressed_kv_cla__decode_kernel(
    A_x, A_k_cache, A_v_cache, A_wq, A_wo, B_x, B_c_kv, B_w_q, B_w_uk, B_w_uv, B_w_o,
):
    return run(A_x, A_k_cache, A_v_cache, A_wq, A_wo, B_x, B_c_kv, B_w_q, B_w_uk, B_w_uv, B_w_o)
```

```python
import jax
import jax.numpy as jnp
from jax import lax
import jax.experimental.pallas as pl
import jax.experimental.pallas.tpu as pltpu

BF16 = jnp.bfloat16
F32 = jnp.float32

H = 32
DH = 128
DM = 512
SK = 4096
WIN = min(4096, max(256, SK // 4))
DC = 512
G = 16
KC = 512

NS, NT = 8, 16
STREAMS = (0, 4, 2, 6, 1, 5, 3, 7)
OPENING_PIECES = 28
CLOSING_PIECES = 16
WO_MXU_STEPS = (4, 4, 4, 2, 1)
WO_VPU_PIECES = (2, 2, 2, 2)

(SEM_X, SEM_BQ, SEM_UK, SEM_WQ, SEM_C, SEM_K0, SEM_K1, SEM_V0, SEM_V1, SEM_UV, SEM_BO,
 SEM_WO_MXU) = range(12)
SEM_WO_VPU = SEM_WO_MXU + len(WO_MXU_STEPS)
NUM_SEMS = SEM_WO_VPU + len(WO_VPU_PIECES)


def _dot(a, b):
    return jnp.dot(a, b, preferred_element_type=F32)


def _dot_nt(a, b):
    return lax.dot_general(a, b, (((1,), (1,)), ((), ())), preferred_element_type=F32)


def _aligned(start, size):
    return pl.ds(start if isinstance(start, int) else pl.multiple_of(start, size), size)


def _stream_and_compute(
        xa_hbm, k_hbm, v_hbm, wq_hbm, wo_hbm, xb_hbm, c_hbm, bq_hbm, uk_hbm, uv_hbm, bo_hbm,
        xa, k, v, wq, wo, xb, c, bq, uk, uv, bo,
        xrep_s, qb_s, qabs_s, sb_s, lat_s, ctx_s, qa_s, pa_s, oa_s, operm_s, ocol_s, out_s,
        sems):
    def rows(src, dst, n):
        def piece(s, t):
            r = _aligned((s * NT + t) * n, n)
            return src.at[r], dst.at[r]
        return piece

    def up_projection(src, dst):
        def piece(s, t):
            idx = (s // 2, 4 * (s % 2) + (t >> 2), pl.ds(4 * (t & 3), 4))
            return src.at[idx], dst.at[idx]
        return piece

    def wq_piece(s, t):
        idx = (_aligned(64 * s + 8 * (t >> 1), 8), _aligned(2048 * (t & 1), 2048))
        return wq_hbm.at[idx], wq.at[idx]

    def window(src, dst, g):
        def piece(s, t):
            h, r = G * g + 2 * s + (t & 1), 128 * (t >> 1)
            return src.at[0, h, _aligned(SK - WIN + r, 128)], dst.at[h, _aligned(r, 128)]
        return piece

    pairs = (
        ((rows(bq_hbm, bq, 4), SEM_BQ), (up_projection(uk_hbm, uk), SEM_UK)),
        ((wq_piece, SEM_WQ), (rows(c_hbm.at[0], c, 32), SEM_C)),
        ((window(k_hbm, k, 0), SEM_K0), (window(v_hbm, v, 0), SEM_V0)),
        ((window(k_hbm, k, 1), SEM_K1), (window(v_hbm, v, 1), SEM_V1)),
        ((up_projection(uv_hbm, uv), SEM_UV), (rows(bo_hbm, bo, 32), SEM_BO)),
    )

    def feed(pair, t, streams=STREAMS):
        for j, s in enumerate(streams):
            for side, (piece, sem) in enumerate(pairs[pair]):
                opening = isinstance(t, int) and pair == 0 and 2 * (t * NS + j) + side < OPENING_PIECES
                pltpu.make_async_copy(*piece(s, t), sems.at[sem]).start(priority=1 if opening else side)

    def feed_wo(sem, t, j0=0, streams=STREAMS):
        for j, s in enumerate(streams):
            closing = isinstance(t, int) and t * NS + j0 + j >= NT * NS - CLOSING_PIECES
            pltpu.make_async_copy(
                wo_hbm.at[_aligned((s * NT + t) * 32, 32)], wo.at[t, j0 + j], sems.at[sem],
            ).start(priority=1 if closing else j % 2)

    def half(i):
        return [STREAMS[j] + (STREAMS[4 + j] - STREAMS[j]) * (i & 1) for j in range(4)]

    def wait(buf, sem):
        pltpu.make_async_copy(buf, buf, sems.at[sem]).wait()

    def loop(feed_step, body, init, trips=8):
        def step(i, carry):
            feed_step(i)
            return body(i, carry)
        return lax.fori_loop(0, trips, step, init)

    xb_dma = pltpu.make_async_copy(xb_hbm, xb, sems.at[SEM_X])
    xa_dma = pltpu.make_async_copy(xa_hbm, xa, sems.at[SEM_X])
    unrolled = pl.cdiv(OPENING_PIECES, 2 * NS)
    for t in range(unrolled):
        feed(0, t)
    loop(lambda i: feed(0, unrolled + i), lambda i, carry: carry, 0, NT - unrolled)
    xb_dma.start()
    xa_dma.start()
    loop(lambda i: feed(1, i), lambda i, carry: carry, 0)

    row = lax.broadcasted_iota(jnp.int32, (G, 128), 0)
    lane = lax.broadcasted_iota(jnp.int32, (G, 128), 1)
    diag = (lane & (G - 1)) == row
    scale = DH ** -0.5

    wait(bq, SEM_BQ)
    xb_dma.wait()
    xa_dma.wait()
    x = xb[0].astype(F32)
    picked = jnp.concatenate(
        [jnp.where((lane >> 3) == row, jnp.broadcast_to(x[:, 128 * b:128 * (b + 1)], (G, 128)), 0.0)
         for b in range(DM // 128)], axis=0).astype(BF16)
    src_lane = lax.broadcasted_iota(jnp.int32, (128, 128), 0)
    dst_lane = lax.broadcasted_iota(jnp.int32, (128, 128), 1)
    spread = jnp.where((src_lane & 7) == (dst_lane >> 4), 1.0, 0.0).astype(BF16)
    xrep_s[...] = _dot(picked, spread)

    def bq_body(i, acc):
        lhs = jnp.concatenate(
            [jnp.where(diag, jnp.broadcast_to(xrep_s[pl.ds(8 * i + u, 1), :], (G, 128)), 0.0).astype(BF16)
             for u in range(8)], axis=1)
        return tuple(
            acc[g] + _dot(lhs, bq[_aligned(64 * i, 64), G * g:G * (g + 1), :].reshape(64 * G, DH))
            for g in range(2))

    qb = loop(lambda i: feed(1, 8 + i), bq_body, (jnp.zeros((G, DH), F32),) * 2)
    for g in range(2):
        qb_s[g] = qb[g].astype(BF16)

    wait(uk, SEM_UK)

    def qabs_body(i, carry):
        b, g = i >> 1, i & 1
        heads = _aligned(G * g, G)
        q = qb_s[g]
        acc = jnp.zeros((G, 128), F32)
        for t in range(16):
            part = jnp.where(diag, _dot_nt(q, uk[b, :, t, heads, :].reshape(128, DH)), 0.0)
            acc = acc + (pltpu.roll(part, t, 1) if t else part)
        for bit in (1, 2, 4, 8):
            acc = jnp.where((row & bit) != 0, pltpu.roll(acc, 128 - bit, 1), acc)
        qabs_s[b, heads, :] = acc.astype(BF16)
        return carry

    loop(lambda i: feed(2, i), qabs_body, 0)

    wait(wq, SEM_WQ)
    xa_rows = jnp.broadcast_to(xa[0].astype(F32), (G, DM)).astype(BF16)

    def qa_body(i, carry):
        q = _dot(xa_rows, wq[:, _aligned(4 * DH * i, 4 * DH)])
        for u in range(4):
            qa_s[4 * i + u] = q[:, DH * u:DH * (u + 1)].astype(BF16)
        return carry

    loop(lambda i: feed(2, 8 + i), qa_body, 0)

    wait(c, SEM_C)
    qabs = jnp.concatenate([qabs_s[b] for b in range(DC // 128)], axis=1)

    def scores_body(i, m):
        s = _dot_nt(qabs, c[_aligned(KC * i, KC), :]) * scale
        sb_s[i] = s
        for u in range(KC // 128):
            m = jnp.maximum(m, s[:, 128 * u:128 * (u + 1)])
        return m

    m = loop(lambda i: feed(3, i >> 1, half(i)), scores_body, jnp.full((H, 128), -jnp.inf, F32))
    m = jnp.max(m, axis=1, keepdims=True)

    def latent_body(i, carry):
        denom, acc = carry
        p = jnp.exp(sb_s[i] - m)
        for u in range(KC // 128):
            denom = denom + p[:, 128 * u:128 * (u + 1)]
        return denom, acc + _dot(p.astype(BF16), c[_aligned(KC * i, KC), :])

    denom, acc = loop(lambda i: feed(3, 4 + (i >> 1), half(i)), latent_body,
                      (jnp.zeros((H, 128), F32), jnp.zeros((H, DC), F32)))
    lat = acc / jnp.sum(denom, axis=1, keepdims=True)
    for b in range(DC // 128):
        for g in range(2):
            lat_s[b, G * g:G * (g + 1), :] = pltpu.roll(
                lat[G * g:G * (g + 1), 128 * b:128 * (b + 1)], 0, 1, stride=1, stride_axis=0)

    for g, sem, feed_step in ((0, SEM_K0, lambda i: feed(3, 8 + i)), (1, SEM_K1, lambda i: feed(4, i))):
        wait(k.at[pl.ds(G * g, G)], sem)

        def sa_body(i, carry, g=g):
            for u in range(2):
                h = G * g + 2 * i + u
                pa_s[pl.ds(h, 1), :] = _dot_nt(qa_s[h], k[h])[0:1, :]
            return carry

        loop(feed_step, sa_body, 0)
        s = pa_s[G * g:G * (g + 1), :] * scale
        p = jnp.exp(s - jnp.max(s, axis=1, keepdims=True))
        pa_s[G * g:G * (g + 1), :] = p / jnp.sum(p, axis=1, keepdims=True)

    for g, sem, feed_step in ((0, SEM_V0, lambda i: feed(4, 8 + i)),
                              (1, SEM_V1, lambda i: feed_wo(SEM_WO_MXU + (i >> 2), i))):
        wait(v.at[pl.ds(G * g, G)], sem)
        p = pa_s[G * g:G * (g + 1), :].astype(BF16)

        def oa_body(i, o, g=g, p=p):
            for u in range(2):
                j = 2 * i + u
                o = jnp.where(row == j, _dot(p, v[G * g + j]), o)
            return o

        oa_s[G * g:G * (g + 1), :] = loop(feed_step, oa_body, jnp.zeros((G, DH), F32))

    def operm_body(u, carry):
        for blk in range(2):
            heads = [jnp.broadcast_to(oa_s[pl.ds(4 * STREAMS[4 * blk + j] + u, 1), :], (G, DH))
                     for j in range(4)]
            for quarter in range(4):
                merged = None
                for j in range(4):
                    shift = (32 * (j - quarter)) % 128
                    moved = pltpu.roll(heads[j], shift, 1) if shift else heads[j]
                    merged = moved if merged is None else jnp.where((lane >> 5) == j, moved, merged)
                operm_s[4 * u + quarter, :, 128 * blk:128 * (blk + 1)] = merged.astype(BF16)
        return carry

    lax.fori_loop(0, NT // 4, operm_body, 0)
    last = operm_s[NT - 1].astype(F32)[0:1, :]
    for blk in range(2):
        ocol_s[128 * blk:128 * (blk + 1), :] = jnp.broadcast_to(
            last[:, 128 * blk:128 * (blk + 1)], (128, 128)).T

    wait(uv, SEM_UV)
    ctx_s[...] = jnp.zeros((H, DH), F32)

    def ctx_body(i, carry):
        b, g = i >> 1, i & 1
        heads = _aligned(G * g, G)
        skewed = lat_s[b, heads, :]
        acc = ctx_s[heads, :]
        for t in range(16):
            shifted = pltpu.roll(skewed, 128 - t, 1) if t else skewed
            acc = acc + _dot(jnp.where(diag, shifted, 0.0).astype(BF16),
                             uv[b, :, t, heads, :].reshape(128, DH))
        ctx_s[heads, :] = acc
        return carry

    loop(lambda i: None, ctx_body, 0)

    wait(bo, SEM_BO)

    def bo_body(i, acc):
        lhs = jnp.concatenate(
            [jnp.broadcast_to(ctx_s[pl.ds(4 * i + u, 1), :], (G, DH)).astype(BF16) for u in range(4)],
            axis=1)
        return acc + _dot(lhs, bo[_aligned(4 * DH * i, 4 * DH), :])

    acc = loop(lambda i: feed_wo(SEM_WO_MXU + 2, 8 + (i >> 1), 4 * (i & 1), half(i)),
               bo_body, jnp.zeros((G, DM), F32))
    assert WO_MXU_STEPS[:3] == (4, 4, 4) and sum(WO_MXU_STEPS) == NT - 1 and sum(WO_VPU_PIECES) == NS
    t0 = 12
    for i, n in enumerate(WO_MXU_STEPS[3:]):
        for t in range(t0, t0 + n):
            feed_wo(SEM_WO_MXU + 3 + i, t)
        t0 += n
    j0 = 0
    for i, n in enumerate(WO_VPU_PIECES):
        feed_wo(SEM_WO_VPU + i, NT - 1, j0, STREAMS[j0:j0 + n])
        j0 += n
    out_s[0, :, DM:2 * DM] = acc[0:1, :].astype(BF16)

    acc = jnp.zeros((G, DM), F32)
    t0 = 0
    for i, n in enumerate(WO_MXU_STEPS):
        wait(wo.at[pl.ds(t0, n)], SEM_WO_MXU + i)
        lhs = jnp.concatenate([operm_s[t] for t in range(t0, t0 + n)], axis=1)
        acc = acc + _dot(lhs, wo[t0:t0 + n].reshape(n * NS * 32, DM))
        t0 += n
    partial = []
    j0 = 0
    for i, n in enumerate(WO_VPU_PIECES):
        if i == len(WO_VPU_PIECES) - 1:
            first_row = lax.broadcasted_iota(jnp.int32, (8, DM), 0) == 0
            partial = [partial[0] + jnp.where(first_row, acc[0:8, :], 0.0)]
        wait(wo.at[NT - 1, pl.ds(j0, n)], SEM_WO_VPU + i)
        ocol = ocol_s[32 * j0:32 * (j0 + n), :]
        prod = (wo[NT - 1, j0:j0 + n].reshape(32 * n, DM).astype(F32)
                * jnp.concatenate([ocol] * (DM // 128), axis=1))
        partial = [prod[8 * u:8 * (u + 1), :] for u in range(4 * n)] + partial
        while len(partial) > 1:
            partial = [partial[u] + partial[u + 1] if u + 1 < len(partial) else partial[u]
                       for u in range(0, len(partial), 2)]
        j0 += n
    out_s[0, :, 0:DM] = jnp.sum(partial[0], axis=0, keepdims=True).astype(BF16)


def _kernel(*refs):
    inputs, out_hbm, scratch, out_sem = refs[:11], refs[11], refs[12:-1], refs[-1]
    out_dma = pltpu.make_async_copy(scratch[-1], out_hbm, out_sem)

    def scoped(sems):
        _stream_and_compute(*inputs, *scratch, sems)
        out_dma.start()

    pl.run_scoped(scoped, pltpu.SemaphoreType.DMA((NUM_SEMS,)))
    out_dma.wait()


@jax.jit
def pallas_concat_heads__sliding_block_cached__compressed_kv_cla__decode_kernel(
    A_x: jax.Array,
    A_k_cache: jax.Array,
    A_v_cache: jax.Array,
    A_wq: jax.Array,
    A_wo: jax.Array,
    B_x: jax.Array,
    B_c_kv: jax.Array,
    B_w_q: jax.Array,
    B_w_uk: jax.Array,
    B_w_uv: jax.Array,
    B_w_o: jax.Array,
):
    assert A_x.shape == B_x.shape == (1, 1, DM)
    assert A_k_cache.shape == A_v_cache.shape == (1, H, SK, DH)
    assert B_c_kv.shape == (1, SK, DC)
    up_shape = (DC // 128, 8, 16, H, DH)
    hbm = pl.BlockSpec(memory_space=pltpu.HBM)

    return pl.pallas_call(
        _kernel,
        out_shape=jax.ShapeDtypeStruct((1, 1, 2 * DM), BF16),
        in_specs=[hbm] * 11,
        out_specs=hbm,
        scratch_shapes=[
            pltpu.VMEM((1, 1, DM), BF16),
            pltpu.VMEM((H, WIN, DH), BF16),
            pltpu.VMEM((H, WIN, DH), BF16),
            pltpu.VMEM((DM, H * DH), BF16),
            pltpu.VMEM((NT, NS, 32, DM), BF16),
            pltpu.VMEM((1, 1, DM), BF16),
            pltpu.VMEM((SK, DC), BF16),
            pltpu.VMEM((DM, H, DH), BF16),
            pltpu.VMEM(up_shape, BF16),
            pltpu.VMEM(up_shape, BF16),
            pltpu.VMEM((H * DH, DM), BF16),
            pltpu.VMEM((DM // 8, 128), F32),
            pltpu.VMEM((2, G, DH), BF16),
            pltpu.VMEM((DC // 128, H, 128), BF16),
            pltpu.VMEM((SK // KC, H, KC), F32),
            pltpu.VMEM((DC // 128, H, 128), F32),
            pltpu.VMEM((H, DH), F32),
            pltpu.VMEM((H, G, DH), BF16),
            pltpu.VMEM((H, WIN), F32),
            pltpu.VMEM((H, DH), F32),
            pltpu.VMEM((NT, G, NS * 32), BF16),
            pltpu.VMEM((NS * 32, 128), F32),
            pltpu.VMEM((1, 1, 2 * DM), BF16),
            pltpu.SemaphoreType.DMA(()),
        ],
        compiler_params=pltpu.CompilerParams(vmem_limit_bytes=64 * 1024 * 1024),
    )(
        A_x, A_k_cache, A_v_cache, A_wq, A_wo, B_x, B_c_kv, B_w_q,
        B_w_uk.reshape(up_shape), B_w_uv.reshape(up_shape), B_w_o.reshape(H * DH, DM),
    )
```
